```python
import os as _os
_os.environ.setdefault("JAX_PLATFORMS", "cpu")
import jax
import jax.numpy as jnp

def _softmax(x, axis=-1):
    return jax.nn.softmax(x, axis=axis)
def _gelu(x):
    return jax.nn.gelu(x, approximate=True)
def _silu(x):
    return jax.nn.silu(x)
def _sigmoid(x):
    return jax.nn.sigmoid(x)
def _layernorm(x, axis=-1, eps=1e-5):
    m = jnp.mean(x, axis=axis, keepdims=True)
    v = jnp.var(x, axis=axis, keepdims=True)
    return (x - m) / jnp.sqrt(v + eps)
def _scatter_add(tgt, idx, src, axis=0):
    return tgt.at[idx].add(src)
def _segment_sum(src, seg, n):
    return jax.ops.segment_sum(src, seg, n)
class _Rng:
    def __init__(self, key):
        self._k = key
    def _next(self):
        self._k, sub = jax.random.split(self._k)
        return sub
    def normal(self, shape):
        return jax.random.normal(self._next(), shape, dtype=jnp.bfloat16)
    def randint(self, lo, hi, shape):
        return jax.random.randint(self._next(), shape, lo, hi, dtype=jnp.int32)
    def uniform(self, shape, lo=0.0, hi=1.0):
        return jax.random.uniform(self._next(), shape, jnp.bfloat16, lo, hi)
    def permutation(self, n):
        return jax.random.permutation(self._next(), n)


kernel_name = 'standalone__gqa_block_cached__near_ridge'

def setup_inputs():
    _rng = _Rng(jax.random.key(int.from_bytes(__import__("os").urandom(4), "little")))
    _w = (lambda a: (lambda t: t.astype(jnp.bfloat16) if jnp.issubdtype(t.dtype, jnp.floating) else t)(jnp.asarray(a)))
    B, Sq, D = 8, 80, 512
    Hq, Hkv, Sk, Dh = 32, 8, 2048, 128
    assert Hq % Hkv == 0, (Hq, Hkv)
    return {
        "x": _w((lambda *s: _rng.normal(s) * 0.8)(B, Sq, D)),
        "k_cache": _w((lambda *s: _rng.normal(s) * 0.8)(B, Hkv, Sk, Dh)),
        "v_cache": _w((lambda *s: _rng.normal(s) * 0.05)(B, Hkv, Sk, Dh)),
        "wq": _w((lambda *s: _rng.normal(s) * 0.8)(D, Hq * Dh) * (D ** -0.5)),
        "wo": _w((lambda *s: _rng.normal(s) * 0.05)(Hq * Dh, D) * ((Hq * Dh) ** -0.5)),
    }

def reference(x, k_cache, v_cache, wq, wo):
    B, Sq, D = x.shape
    Hq, Dh = 32, 128
    Hkv = k_cache.shape[1]
    rep = Hq // Hkv
    q = (lambda x, *d: x.transpose(*d))((x @ wq).reshape(B, Sq, Hq, Dh), 0, 2, 1, 3)
    k = jnp.repeat(k_cache, rep, axis=1)
    v = jnp.repeat(v_cache, rep, axis=1)
    scores = jnp.einsum("bhqd,bhkd->bhqk", q, k) * (Dh ** -0.5)
    p = _softmax(scores, axis=-1)
    o = jnp.einsum("bhqk,bhkd->bhqd", p, v)
    return (lambda x, *d: x.transpose(*d))(o, 0, 2, 1, 3).reshape(B, Sq, Hq * Dh) @ wo
```

```python
import jax
import jax.numpy as jnp
import numpy as np
from jax.experimental import pallas as pl
from jax.experimental.pallas import tpu as pltpu

HQ, DH = 32, 128
LANES = 128
_NT = (((1,), (1,)), ((), ()))

WQ_CUTS = (0, 128, 512, 1536, 4096)
MID = 2
QN = 512
ON = 128
LAG = 2


@jax.jit
def pallas_standalone__gqa_block_cached__near_ridge_kernel(
    x: jax.Array,
    k_cache: jax.Array,
    v_cache: jax.Array,
    wq: jax.Array,
    wo: jax.Array,
):
    B, SQ, D = x.shape
    _, HKV, SK, _ = k_cache.shape
    REP = HQ // HKV
    M = REP * SQ
    G = REP * DH
    ROWS = B * SQ
    nq = len(WQ_CUTS) - 1
    no = D // ON
    q_scale = float(DH**-0.5 * np.log2(np.e))
    bf16, f32 = jnp.bfloat16, jnp.float32

    def kernel(
        zero_ref, x_hbm, k_hbm, v_hbm, wq_hbm, wo_hbm, o_hbm,
        x_s, k_s, v_s, wq_s, wo_s, q_s, acc_s, o_s, co_s, cl_s, sem,
    ):
        s_k, s_v, s_w = 0, HKV, 2 * HKV
        s_q = 3 * HKV
        s_o = s_q + nq
        s_m = s_o + no

        def k_copy(h, a=0, b=B, s=None):
            return pltpu.make_async_copy(
                k_hbm.at[pl.ds(a, b - a), h], k_s.at[h, pl.ds(a, b - a)],
                sem.at[s_k + h if s is None else s])

        def v_copy(h, a=0, b=B, s=None):
            return pltpu.make_async_copy(
                v_hbm.at[pl.ds(a, b - a), h], v_s.at[h, pl.ds(a, b - a)],
                sem.at[s_v + h if s is None else s])

        def wo_copy(h):
            return pltpu.make_async_copy(wo_hbm.at[h], wo_s.at[h], sem.at[s_w + h])

        x_copy = pltpu.make_async_copy(x_hbm, x_s, sem.at[s_m])
        wq_copies = [
            pltpu.make_async_copy(
                wq_hbm.at[:, pl.ds(a, b - a)], wq_s.at[:, pl.ds(a, b - a)], sem.at[s_q + i])
            for i, (a, b) in enumerate(zip(WQ_CUTS[:-1], WQ_CUTS[1:]))
        ]
        o_copies = [
            pltpu.make_async_copy(
                o_s.at[:, pl.ds(j * ON, ON)], o_hbm.at[:, pl.ds(j * ON, ON)], sem.at[s_o + j])
            for j in range(no)
        ]
        k_head, v_head = k_copy(0, 0, MID + 1, s_m + 1), v_copy(0, 0, MID, s_m + 2)
        k_rest, v_rest = k_copy(0, MID + 1, B), v_copy(0, MID, B)

        for c in (x_copy, *wq_copies, k_head, v_head, k_rest, v_rest, wo_copy(0)):
            c.start()

        x_copy.wait()
        for i, (a, b) in enumerate(zip(WQ_CUTS[:-1], WQ_CUTS[1:])):
            wq_copies[i].wait()
            for n0 in range(a, b, QN):
                n1 = min(n0 + QN, b)
                q = jnp.dot(x_s[...], wq_s[:, n0:n1], preferred_element_type=f32)
                q = (q * q_scale).astype(bf16)
                for t in range((n1 - n0) // DH):
                    h, r = divmod(n0 // DH + t, REP)
                    for bb in range(B):
                        q_s[h, bb, r * SQ:(r + 1) * SQ, :] = (
                            q[bb * SQ:(bb + 1) * SQ, t * DH:(t + 1) * DH])

        def normalise(o, lane_sum):
            l = jnp.sum(lane_sum, axis=-1, keepdims=True)
            r = pl.reciprocal(l, approx=True)
            r = r * (2.0 - l * r)
            return (o * r).astype(bf16)

        def lane_fold(op, a):
            out = a[:, :LANES]
            for j in range(1, SK // LANES):
                out = op(out, a[:, j * LANES:(j + 1) * LANES])
            return out

        def attend(h, mid_wait=None):
            hz = h + zero_ref[0]
            pending = {}
            for p in range(B):
                s = jax.lax.dot_general(q_s[h, p], k_s[h, p], _NT, preferred_element_type=f32)
                lane_max = lane_fold(jnp.maximum, s)
                if p >= LAG:
                    o, _ = pending.pop(p - LAG)
                    lane_sum = pltpu.bitcast(v_s[hz, p - LAG, M:3 * M, :], f32)
                    v_s[hz, p - LAG, 0:M, :] = normalise(o, lane_sum)
                if 1 <= p <= B - LAG:
                    v_s[hz, p - 1, M:3 * M, :] = pltpu.bitcast(pending[p - 1][1], bf16)
                if mid_wait is not None and p == MID:
                    mid_wait()
                e = jnp.exp2(s - jnp.max(lane_max, axis=-1, keepdims=True))
                o = jnp.dot(e.astype(bf16), v_s[h, p], preferred_element_type=f32)
                pending[p] = (o, lane_fold(jnp.add, e))
            for p, (o, lane_sum) in pending.items():
                if p == B - 1:
                    co_s[...] = o
                    cl_s[...] = lane_sum
                else:
                    v_s[hz, p, 0:M, :] = normalise(o, lane_sum)

        def project(h, last):
            tail = normalise(co_s[...], cl_s[...])

            def piece(p, r):
                if p == B - 1:
                    return tail[r * SQ:(r + 1) * SQ, :]
                return v_s[h, p, r * SQ:(r + 1) * SQ, :]

            a = jnp.concatenate(
                [jnp.concatenate([piece(p, r) for p in range(B)], axis=0) for r in range(REP)],
                axis=1)
            for j in range(no):
                cols = slice(j * ON, (j + 1) * ON)
                y = acc_s[:, cols] + jnp.dot(a, wo_s[h, :, cols], preferred_element_type=f32)
                if last:
                    o_s[:, cols] = y.astype(bf16)
                    o_copies[j].start()
                else:
                    acc_s[:, cols] = y

        k_head.wait()
        v_head.wait()
        for c in (k_copy(1), v_copy(1), wo_copy(1)):
            c.start()
        acc_s[...] = jnp.zeros_like(acc_s)

        def wait_rest():
            k_rest.wait()
            v_rest.wait()

        attend(0, wait_rest)

        def body(h, carry):
            k_copy(h).wait()
            v_copy(h).wait()
            wo_copy(h - 1).wait()

            @pl.when(h + 1 < HKV)
            def _():
                for c in (k_copy(h + 1), v_copy(h + 1), wo_copy(h + 1)):
                    c.start()

            project(h - 1, False)
            attend(h)
            return carry

        jax.lax.fori_loop(1, HKV, body, None)
        wo_copy(HKV - 1).wait()
        project(HKV - 1, True)
        for c in o_copies:
            c.wait()

    any_spec = pl.BlockSpec(memory_space=pl.ANY)
    out = pl.pallas_call(
        kernel,
        in_specs=[pl.BlockSpec(memory_space=pltpu.SMEM)] + [any_spec] * 5,
        out_specs=any_spec,
        out_shape=jax.ShapeDtypeStruct((ROWS, D), x.dtype),
        scratch_shapes=[
            pltpu.VMEM((ROWS, D), bf16),
            pltpu.VMEM((HKV, B, SK, DH), bf16),
            pltpu.VMEM((HKV, B, SK, DH), bf16),
            pltpu.VMEM((D, HQ * DH), bf16),
            pltpu.VMEM((HKV, G, D), bf16),
            pltpu.VMEM((HKV, B, M, DH), bf16),
            pltpu.VMEM((ROWS, D), f32),
            pltpu.VMEM((ROWS, D), bf16),
            pltpu.VMEM((M, DH), f32),
            pltpu.VMEM((M, DH), f32),
            pltpu.SemaphoreType.DMA((3 * HKV + nq + no + 3,)),
        ],
        compiler_params=pltpu.CompilerParams(vmem_limit_bytes=120 * 2**20),
    )(
        jnp.zeros((1,), jnp.int32),
        x.reshape(ROWS, D),
        k_cache,
        v_cache,
        wq,
        wo.reshape(HKV, G, D),
    )
    return out.reshape(B, SQ, D)
```

```python
import jax
import jax.numpy as jnp
import numpy as np
from jax.experimental import pallas as pl
from jax.experimental.pallas import tpu as pltpu

HQ, DH = 32, 128
LANES = 128
_NT = (((1,), (1,)), ((), ()))

WQ_CUTS = (0, 128, 512, 1536, 4096)
QN = 512
HEAD = 2
CHUNKS = (1, 3, 4)
LAST_CHUNKS = (1,) * 8


@jax.jit
def pallas_standalone__gqa_block_cached__near_ridge_kernel(
    x: jax.Array,
    k_cache: jax.Array,
    v_cache: jax.Array,
    wq: jax.Array,
    wo: jax.Array,
):
    B, SQ, D = x.shape
    _, HKV, SK, _ = k_cache.shape
    REP = HQ // HKV
    M = REP * SQ
    G = REP * DH
    ROWS = B * SQ
    q_scale = float(DH**-0.5 * np.log2(np.e))
    bf16, f32 = jnp.bfloat16, jnp.float32

    sem_k, sem_v, sem_wo = 0, HKV, 2 * HKV
    sem_wq = 3 * HKV
    sem_out = sem_wq + len(WQ_CUTS) - 1
    sem_misc = sem_out + len(LAST_CHUNKS)
    num_sems = sem_misc + 3

    def kernel(
        x_hbm, k_hbm, v_hbm, wq_hbm, wo_hbm, o_hbm,
        x_s, k_s, v_s, wq_s, wo_s, q_s, acc_s, o_s, first_s, pv_s, sum_s, sem,
    ):
        def kv_copy(hbm, vmem, s, h, b0=0, b1=B):
            return pltpu.make_async_copy(
                hbm.at[pl.ds(b0, b1 - b0), h], vmem.at[h, pl.ds(b0, b1 - b0)], sem.at[s])

        def head_copies(h):
            return (
                kv_copy(k_hbm, k_s, sem_k + h, h),
                kv_copy(v_hbm, v_s, sem_v + h, h),
                pltpu.make_async_copy(wo_hbm.at[h], wo_s.at[h], sem.at[sem_wo + h]),
            )

        x_copy = pltpu.make_async_copy(x_hbm, x_s, sem.at[sem_misc])
        wq_copies = [
            pltpu.make_async_copy(
                wq_hbm.at[:, pl.ds(a, b - a)], wq_s.at[:, pl.ds(a, b - a)], sem.at[sem_wq + i])
            for i, (a, b) in enumerate(zip(WQ_CUTS[:-1], WQ_CUTS[1:]))
        ]
        kv_head = (
            kv_copy(k_hbm, k_s, sem_misc + 1, 0, 0, HEAD),
            kv_copy(v_hbm, v_s, sem_misc + 2, 0, 0, HEAD),
        )
        kv_rest = (
            kv_copy(k_hbm, k_s, sem_k, 0, HEAD, B),
            kv_copy(v_hbm, v_s, sem_v, 0, HEAD, B),
        )
        out_copies = []
        b0 = 0
        for j, n in enumerate(LAST_CHUNKS):
            rows = pl.ds(b0 * SQ, n * SQ)
            out_copies.append(
                pltpu.make_async_copy(o_s.at[rows], o_hbm.at[rows], sem.at[sem_out + j]))
            b0 += n

        for c in (x_copy, *wq_copies, *kv_head, *kv_rest, head_copies(0)[2]):
            c.start()
        acc_s[...] = jnp.zeros_like(acc_s)

        x_copy.wait()
        for i, (a, b) in enumerate(zip(WQ_CUTS[:-1], WQ_CUTS[1:])):
            wq_copies[i].wait()
            for n0 in range(a, b, QN):
                n1 = min(n0 + QN, b)
                q = jnp.dot(x_s[...], wq_s[:, n0:n1], preferred_element_type=f32)
                q = (q * q_scale).astype(bf16)
                for t in range((n1 - n0) // DH):
                    h, r = divmod(n0 // DH + t, REP)
                    for bb in range(B):
                        q_s[h, bb, r * SQ:(r + 1) * SQ, :] = (
                            q[bb * SQ:(bb + 1) * SQ, t * DH:(t + 1) * DH])

        def lane_fold(op, a):
            out = a[:, :LANES]
            for j in range(1, SK // LANES):
                out = op(out, a[:, j * LANES:(j + 1) * LANES])
            return out

        def normalise(pv, lane_sum):
            total = jnp.sum(lane_sum, axis=-1, keepdims=True)
            inv = pl.reciprocal(total, approx=True)
            inv = inv * (2.0 - total * inv)
            return (pv * inv).astype(bf16)

        def attend(h, wait_rest=False):
            for b in range(B):
                if wait_rest and b == HEAD:
                    for c in kv_rest:
                        c.wait()
                s = jax.lax.dot_general(q_s[h, b], k_s[h, b], _NT, preferred_element_type=f32)
                row_max = jnp.max(lane_fold(jnp.maximum, s), axis=-1, keepdims=True)
                e = jnp.exp2(s - row_max)
                lane_sum = lane_fold(jnp.add, e)
                pv = jnp.dot(e.astype(bf16), v_s[h, b], preferred_element_type=f32)
                if b == 0:
                    first = (pv, lane_sum)
                else:
                    pv_s[b - 1] = pv
                    sum_s[b - 1] = lane_sum
            first_s[...] = normalise(*first)

        def project(h, chunks, last):
            b0 = 0
            for j, n in enumerate(chunks):
                outs = [
                    first_s[...] if b == 0 else normalise(pv_s[b - 1], sum_s[b - 1])
                    for b in range(b0, b0 + n)
                ]
                a = jnp.concatenate(
                    [jnp.concatenate([o[r * SQ:(r + 1) * SQ, :] for o in outs], axis=0)
                     for r in range(REP)],
                    axis=1)
                rows = slice(b0 * SQ, (b0 + n) * SQ)
                y = acc_s[rows, :] + jnp.dot(a, wo_s[h], preferred_element_type=f32)
                if last:
                    o_s[rows, :] = y.astype(o_s.dtype)
                    out_copies[j].start()
                else:
                    acc_s[rows, :] = y
                b0 += n

        for c in kv_head:
            c.wait()
        for c in head_copies(1):
            c.start()
        attend(0, wait_rest=True)

        @pl.loop(1, HKV)
        def _(h):
            k_copy, v_copy, _ = head_copies(h)
            k_copy.wait()
            v_copy.wait()
            head_copies(h - 1)[2].wait()
            project(h - 1, CHUNKS, last=False)

            @pl.when(h + 1 < HKV)
            def _():
                for c in head_copies(h + 1):
                    c.start()

            attend(h)

        head_copies(HKV - 1)[2].wait()
        project(HKV - 1, LAST_CHUNKS, last=True)
        for c in out_copies:
            c.wait()

    any_spec = pl.BlockSpec(memory_space=pl.ANY)
    out = pl.pallas_call(
        kernel,
        in_specs=[any_spec] * 5,
        out_specs=any_spec,
        out_shape=jax.ShapeDtypeStruct((ROWS, D), x.dtype),
        scratch_shapes=[
            pltpu.VMEM((ROWS, D), bf16),
            pltpu.VMEM((HKV, B, SK, DH), bf16),
            pltpu.VMEM((HKV, B, SK, DH), bf16),
            pltpu.VMEM((D, HQ * DH), bf16),
            pltpu.VMEM((HKV, G, D), bf16),
            pltpu.VMEM((HKV, B, M, DH), bf16),
            pltpu.VMEM((ROWS, D), f32),
            pltpu.VMEM((ROWS, D), x.dtype),
            pltpu.VMEM((M, DH), bf16),
            pltpu.VMEM((B - 1, M, DH), f32),
            pltpu.VMEM((B - 1, M, LANES), f32),
            pltpu.SemaphoreType.DMA((num_sems,)),
        ],
        compiler_params=pltpu.CompilerParams(vmem_limit_bytes=120 * 2**20),
    )(x.reshape(ROWS, D), k_cache, v_cache, wq, wo.reshape(HKV, G, D))
    return out.reshape(B, SQ, D)
```

```python
import jax
import jax.numpy as jnp
import numpy as np
from jax.experimental import pallas as pl
from jax.experimental.pallas import tpu as pltpu

HQ, DH = 32, 128
LANES = 128
_NT = (((1,), (1,)), ((), ()))

STAGES = ((4, 2), (6, 4), (8, 8), (8, 20), (8, 32))
Q_HEADS = 4
HEAD = 2
CHUNKS = (1, 3, 4)
LAST_CHUNKS = (1,) * 8


@jax.jit
def pallas_standalone__gqa_block_cached__near_ridge_kernel(
    x: jax.Array,
    k_cache: jax.Array,
    v_cache: jax.Array,
    wq: jax.Array,
    wo: jax.Array,
):
    B, SQ, D = x.shape
    _, HKV, SK, _ = k_cache.shape
    REP = HQ // HKV
    M = REP * SQ
    G = REP * DH
    ROWS = B * SQ
    assert STAGES[-1] == (B, HQ) and sum(CHUNKS) == sum(LAST_CHUNKS) == B
    q_scale = float(DH**-0.5 * np.log2(np.e))
    bf16, f32 = jnp.bfloat16, jnp.float32

    sem_k, sem_v, sem_wo = 0, HKV, 2 * HKV
    sem_stage = 3 * HKV
    sem_out = sem_stage + 2 * len(STAGES)
    sem_head = sem_out + len(LAST_CHUNKS)
    num_sems = sem_head + 2

    def kernel(
        x_hbm, k_hbm, v_hbm, wq_hbm, wo_hbm, o_hbm,
        x_s, k_s, v_s, wq_s, wo_s, q_s, acc_s, o_s, first_s, pv_s, sum_s, sem,
    ):
        def kv_copies(h, b0=0, b1=B, k_sem=None, v_sem=None):
            batches = pl.ds(b0, b1 - b0)
            return (
                pltpu.make_async_copy(
                    k_hbm.at[batches, h], k_s.at[h, batches],
                    sem.at[sem_k + h if k_sem is None else k_sem]),
                pltpu.make_async_copy(
                    v_hbm.at[batches, h], v_s.at[h, batches],
                    sem.at[sem_v + h if v_sem is None else v_sem]),
            )

        def wo_copy(h):
            return pltpu.make_async_copy(wo_hbm.at[h], wo_s.at[h], sem.at[sem_wo + h])

        def lane_fold(op, a):
            out = a[:, :LANES]
            for j in range(1, SK // LANES):
                out = op(out, a[:, j * LANES:(j + 1) * LANES])
            return out

        def normalise(pv, lane_sum):
            total = jnp.sum(lane_sum, axis=-1, keepdims=True)
            inv = pl.reciprocal(total, approx=True)
            inv = inv * (2.0 - total * inv)
            return (pv * inv).astype(bf16)

        def project_q(b0, b1, n0, n1):
            q = jnp.dot(
                x_s[b0 * SQ:b1 * SQ, :], wq_s[:, n0 * DH:n1 * DH], preferred_element_type=f32)
            q = (q * q_scale).astype(bf16)
            for n in range(n1 - n0):
                h, r = divmod(n0 + n, REP)
                for b in range(b1 - b0):
                    q_s[h, b0 + b, r * SQ:(r + 1) * SQ, :] = (
                        q[b * SQ:(b + 1) * SQ, n * DH:(n + 1) * DH])

        def attend(h, late_copies=()):
            for b in range(B):
                if b == HEAD:
                    for c in late_copies:
                        c.wait()
                s = jax.lax.dot_general(q_s[h, b], k_s[h, b], _NT, preferred_element_type=f32)
                row_max = jnp.max(lane_fold(jnp.maximum, s), axis=-1, keepdims=True)
                e = jnp.exp2(s - row_max)
                lane_sum = lane_fold(jnp.add, e)
                pv = jnp.dot(e.astype(bf16), v_s[h, b], preferred_element_type=f32)
                if b == 0:
                    first = (pv, lane_sum)
                else:
                    pv_s[b - 1] = pv
                    sum_s[b - 1] = lane_sum
            first_s[...] = normalise(*first)

        def project_out(h, chunks, last):
            out_copies = []
            b0 = 0
            for j, n in enumerate(chunks):
                outs = [
                    first_s[...] if b == 0 else normalise(pv_s[b - 1], sum_s[b - 1])
                    for b in range(b0, b0 + n)
                ]
                a = jnp.concatenate(
                    [jnp.concatenate([o[r * SQ:(r + 1) * SQ, :] for o in outs], axis=0)
                     for r in range(REP)],
                    axis=1)
                rows = pl.ds(b0 * SQ, n * SQ)
                y = acc_s[rows, :] + jnp.dot(a, wo_s[h], preferred_element_type=f32)
                if last:
                    o_s[rows, :] = y.astype(o_s.dtype)
                    c = pltpu.make_async_copy(o_s.at[rows], o_hbm.at[rows], sem.at[sem_out + j])
                    c.start()
                    out_copies.append(c)
                else:
                    acc_s[rows, :] = y
                b0 += n
            for c in out_copies:
                c.wait()

        step = pl.program_id(0)

        @pl.when(step == 0)
        def _():
            stage_copies = []
            b0 = n0 = 0
            for i, (b1, n1) in enumerate(STAGES):
                copies = []
                if n1 > n0:
                    cols = pl.ds(n0 * DH, (n1 - n0) * DH)
                    copies.append(pltpu.make_async_copy(
                        wq_hbm.at[:, cols], wq_s.at[:, cols], sem.at[sem_stage + 2 * i]))
                if b1 > b0:
                    rows = pl.ds(b0 * SQ, (b1 - b0) * SQ)
                    copies.append(pltpu.make_async_copy(
                        x_hbm.at[rows], x_s.at[rows], sem.at[sem_stage + 2 * i + 1]))
                stage_copies.append(copies)
                b0, n0 = b1, n1
            stage_copies[-1] += kv_copies(0, 0, HEAD, sem_head, sem_head + 1)
            kv_rest = kv_copies(0, HEAD, B)

            for copies in (*stage_copies, kv_rest):
                for c in copies:
                    c.start()
            wo_copy(0).start()
            for h in range(1, HKV):
                for c in kv_copies(h):
                    c.start()
                wo_copy(h).start()
            acc_s[...] = jnp.zeros_like(acc_s)

            b0 = n0 = 0
            for copies, (b1, n1) in zip(stage_copies, STAGES):
                for c in copies:
                    c.wait()
                if b1 > b0 and n0 > 0:
                    project_q(b0, b1, 0, n0)
                for n in range(n0, n1, Q_HEADS):
                    project_q(0, b1, n, min(n + Q_HEADS, n1))
                b0, n0 = b1, n1

            attend(0, kv_rest)

        @pl.when(jnp.logical_and(step > 0, step < HKV))
        def _():
            for c in kv_copies(step):
                c.wait()
            wo_copy(step - 1).wait()
            project_out(step - 1, CHUNKS, last=False)
            attend(step)

        @pl.when(step == HKV)
        def _():
            wo_copy(HKV - 1).wait()
            project_out(HKV - 1, LAST_CHUNKS, last=True)

    any_spec = pl.BlockSpec(memory_space=pl.ANY)
    out = pl.pallas_call(
        kernel,
        grid=(HKV + 1,),
        in_specs=[any_spec] * 5,
        out_specs=any_spec,
        out_shape=jax.ShapeDtypeStruct((ROWS, D), x.dtype),
        scratch_shapes=[
            pltpu.VMEM((ROWS, D), bf16),
            pltpu.VMEM((HKV, B, SK, DH), bf16),
            pltpu.VMEM((HKV, B, SK, DH), bf16),
            pltpu.VMEM((D, HQ * DH), bf16),
            pltpu.VMEM((HKV, G, D), bf16),
            pltpu.VMEM((HKV, B, M, DH), bf16),
            pltpu.VMEM((ROWS, D), f32),
            pltpu.VMEM((ROWS, D), x.dtype),
            pltpu.VMEM((M, DH), bf16),
            pltpu.VMEM((B - 1, M, DH), f32),
            pltpu.VMEM((B - 1, M, LANES), f32),
            pltpu.SemaphoreType.DMA((num_sems,)),
        ],
        compiler_params=pltpu.CompilerParams(
            dimension_semantics=("arbitrary",), vmem_limit_bytes=120 * 2**20),
    )(x.reshape(ROWS, D), k_cache, v_cache, wq, wo.reshape(HKV, G, D))
    return out.reshape(B, SQ, D)
```

```python
import functools

import jax
import jax.numpy as jnp
import numpy as np
from jax.experimental import pallas as pl
from jax.experimental.pallas import tpu as pltpu

HQ, DH = 32, 128
LANES = 128
_NT = (((1,), (1,)), ((), ()))

STAGES = ((4, 2), (6, 4), (8, 8), (8, 20), (8, 32))
Q_HEADS = 4
HEAD = 2
CHUNKS = (1, 3, 4)
LAST_CHUNKS = (1,) * 8


@jax.jit
def pallas_standalone__gqa_block_cached__near_ridge_kernel(
    x: jax.Array,
    k_cache: jax.Array,
    v_cache: jax.Array,
    wq: jax.Array,
    wo: jax.Array,
):
    B, SQ, D = x.shape
    _, HKV, SK, _ = k_cache.shape
    REP = HQ // HKV
    M = REP * SQ
    G = REP * DH
    ROWS = B * SQ
    assert STAGES[-1] == (B, HQ) and sum(CHUNKS) == sum(LAST_CHUNKS) == B
    q_scale = float(DH**-0.5 * np.log2(np.e))
    bf16, f32 = jnp.bfloat16, jnp.float32

    sem_k, sem_v, sem_wo = 0, HKV, 2 * HKV
    sem_stage = 3 * HKV
    sem_out = sem_stage + 2 * len(STAGES)
    sem_head = sem_out + len(LAST_CHUNKS)
    num_sems = sem_head + 2

    def kernel(
        x_hbm, k_hbm, v_hbm, wq_hbm, wo_hbm, o_hbm,
        x_s, k_s, v_s, wq_s, wo_s, q_s, acc_s, o_s, first_s, pv_s, sum_s, sem,
    ):
        def kv_copies(h, b0=0, b1=B, k_sem=None, v_sem=None):
            batches = pl.ds(b0, b1 - b0)
            return (
                pltpu.make_async_copy(
                    k_hbm.at[batches, h], k_s.at[h, batches],
                    sem.at[sem_k + h if k_sem is None else k_sem]),
                pltpu.make_async_copy(
                    v_hbm.at[batches, h], v_s.at[h, batches],
                    sem.at[sem_v + h if v_sem is None else v_sem]),
            )

        def wo_copy(h):
            return pltpu.make_async_copy(wo_hbm.at[h], wo_s.at[h], sem.at[sem_wo + h])

        def tiles(a):
            return [a[:, j * LANES:(j + 1) * LANES] for j in range(SK // LANES)]

        def lane_max(a):
            return functools.reduce(jnp.maximum, tiles(a))

        def lane_total(a):
            t = tiles(a)
            return functools.reduce(
                jnp.add,
                [(t[j] + t[j + 1]) + (t[j + 2] + t[j + 3]) for j in range(0, len(t), 4)])

        def normalise(pv, lane_sum):
            total = jnp.sum(lane_sum, axis=-1, keepdims=True)
            inv = pl.reciprocal(total, approx=True)
            inv = inv * (2.0 - total * inv)
            return (pv * inv).astype(bf16)

        def project_q(b0, b1, n0, n1):
            q = jnp.dot(
                x_s[b0 * SQ:b1 * SQ, :], wq_s[:, n0 * DH:n1 * DH], preferred_element_type=f32)
            q = (q * q_scale).astype(bf16)
            for n in range(n1 - n0):
                h, r = divmod(n0 + n, REP)
                for b in range(b1 - b0):
                    q_s[h, b0 + b, r * SQ:(r + 1) * SQ, :] = (
                        q[b * SQ:(b + 1) * SQ, n * DH:(n + 1) * DH])

        def attend(h, late_copies=()):
            for b in range(B):
                if b == HEAD:
                    for c in late_copies:
                        c.wait()
                s = jax.lax.dot_general(q_s[h, b], k_s[h, b], _NT, preferred_element_type=f32)
                row_max = jnp.max(lane_max(s), axis=-1, keepdims=True)
                e = jnp.exp2(s - row_max)
                lane_sum = lane_total(e)
                pv = jnp.dot(e.astype(bf16), v_s[h, b], preferred_element_type=f32)
                if b == 0:
                    first = (pv, lane_sum)
                else:
                    pv_s[b - 1] = pv
                    sum_s[b - 1] = lane_sum
            first_s[...] = normalise(*first)

        def project_out(h, chunks, last):
            out_copies = []
            b0 = 0
            for j, n in enumerate(chunks):
                outs = [
                    first_s[...] if b == 0 else normalise(pv_s[b - 1], sum_s[b - 1])
                    for b in range(b0, b0 + n)
                ]
                a = jnp.concatenate(
                    [jnp.concatenate([o[r * SQ:(r + 1) * SQ, :] for o in outs], axis=0)
                     for r in range(REP)],
                    axis=1)
                rows = pl.ds(b0 * SQ, n * SQ)
                y = acc_s[rows, :] + jnp.dot(a, wo_s[h], preferred_element_type=f32)
                if last:
                    o_s[rows, :] = y.astype(o_s.dtype)
                    c = pltpu.make_async_copy(o_s.at[rows], o_hbm.at[rows], sem.at[sem_out + j])
                    c.start()
                    out_copies.append(c)
                else:
                    acc_s[rows, :] = y
                b0 += n
            for c in out_copies:
                c.wait()

        step = pl.program_id(0)

        @pl.when(step == 0)
        def _():
            stage_copies = []
            b0 = n0 = 0
            for i, (b1, n1) in enumerate(STAGES):
                copies = []
                if n1 > n0:
                    cols = pl.ds(n0 * DH, (n1 - n0) * DH)
                    copies.append(pltpu.make_async_copy(
                        wq_hbm.at[:, cols], wq_s.at[:, cols], sem.at[sem_stage + 2 * i]))
                if b1 > b0:
                    rows = pl.ds(b0 * SQ, (b1 - b0) * SQ)
                    copies.append(pltpu.make_async_copy(
                        x_hbm.at[rows], x_s.at[rows], sem.at[sem_stage + 2 * i + 1]))
                stage_copies.append(copies)
                b0, n0 = b1, n1
            stage_copies[-1] += kv_copies(0, 0, HEAD, sem_head, sem_head + 1)
            kv_rest = kv_copies(0, HEAD, B)

            for copies in (*stage_copies, kv_rest):
                for c in copies:
                    c.start()
            wo_copy(0).start()
            for h in range(1, HKV):
                for c in kv_copies(h):
                    c.start()
                wo_copy(h).start()
            acc_s[...] = jnp.zeros_like(acc_s)

            b0 = n0 = 0
            for copies, (b1, n1) in zip(stage_copies, STAGES):
                for c in copies:
                    c.wait()
                if b1 > b0 and n0 > 0:
                    project_q(b0, b1, 0, n0)
                for n in range(n0, n1, Q_HEADS):
                    project_q(0, b1, n, min(n + Q_HEADS, n1))
                b0, n0 = b1, n1

            attend(0, kv_rest)

        @pl.when(jnp.logical_and(step > 0, step < HKV))
        def _():
            for c in kv_copies(step):
                c.wait()
            wo_copy(step - 1).wait()
            project_out(step - 1, CHUNKS, last=False)
            attend(step)

        @pl.when(step == HKV)
        def _():
            wo_copy(HKV - 1).wait()
            project_out(HKV - 1, LAST_CHUNKS, last=True)

    any_spec = pl.BlockSpec(memory_space=pl.ANY)
    out = pl.pallas_call(
        kernel,
        grid=(HKV + 1,),
        in_specs=[any_spec] * 5,
        out_specs=any_spec,
        out_shape=jax.ShapeDtypeStruct((ROWS, D), x.dtype),
        scratch_shapes=[
            pltpu.VMEM((ROWS, D), bf16),
            pltpu.VMEM((HKV, B, SK, DH), bf16),
            pltpu.VMEM((HKV, B, SK, DH), bf16),
            pltpu.VMEM((D, HQ * DH), bf16),
            pltpu.VMEM((HKV, G, D), bf16),
            pltpu.VMEM((HKV, B, M, DH), bf16),
            pltpu.VMEM((ROWS, D), f32),
            pltpu.VMEM((ROWS, D), x.dtype),
            pltpu.VMEM((M, DH), bf16),
            pltpu.VMEM((B - 1, M, DH), f32),
            pltpu.VMEM((B - 1, M, LANES), f32),
            pltpu.SemaphoreType.DMA((num_sems,)),
        ],
        compiler_params=pltpu.CompilerParams(
            dimension_semantics=("arbitrary",), vmem_limit_bytes=120 * 2**20),
    )(x.reshape(ROWS, D), k_cache, v_cache, wq, wo.reshape(HKV, G, D))
    return out.reshape(B, SQ, D)
```
